```python
import os as _os
_os.environ.setdefault("JAX_PLATFORMS", "cpu")
import jax
import jax.numpy as jnp

def _softmax(x, axis=-1):
    return jax.nn.softmax(x, axis=axis)
def _gelu(x):
    return jax.nn.gelu(x, approximate=True)
def _silu(x):
    return jax.nn.silu(x)
def _sigmoid(x):
    return jax.nn.sigmoid(x)
def _layernorm(x, axis=-1, eps=1e-5):
    m = jnp.mean(x, axis=axis, keepdims=True)
    v = jnp.var(x, axis=axis, keepdims=True)
    return (x - m) / jnp.sqrt(v + eps)
def _scatter_add(tgt, idx, src, axis=0):
    return tgt.at[idx].add(src)
def _segment_sum(src, seg, n):
    return jax.ops.segment_sum(src, seg, n)
class _Rng:
    def __init__(self, key):
        self._k = key
    def _next(self):
        self._k, sub = jax.random.split(self._k)
        return sub
    def normal(self, shape):
        return jax.random.normal(self._next(), shape, dtype=jnp.bfloat16)
    def randint(self, lo, hi, shape):
        return jax.random.randint(self._next(), shape, lo, hi, dtype=jnp.int32)
    def uniform(self, shape, lo=0.0, hi=1.0):
        return jax.random.uniform(self._next(), shape, jnp.bfloat16, lo, hi)
    def permutation(self, n):
        return jax.random.permutation(self._next(), n)


kernel_name = 'standalone__dense_activation_gelu__prompt'

def setup_inputs():
    _rng = _Rng(jax.random.key(int.from_bytes(__import__("os").urandom(4), "little")))
    _w = (lambda a: (lambda t: t.astype(jnp.bfloat16) if jnp.issubdtype(t.dtype, jnp.floating) else t)(jnp.asarray(a)))
    B, S, D, F = 1, 2048, 640, 1728
    return {
        "x": _w((lambda *s: _rng.normal(s) * 0.05)(B, S, D)),
        "w1": _w((lambda *s: _rng.normal(s) * 0.05)(D, F) * (D ** -0.5)),
        "b1": _w((lambda *s: _rng.normal(s) * 0.05)(F) * 0.01),
        "w2": _w((lambda *s: _rng.normal(s) * 0.05)(F, D) * (F ** -0.5)),
        "b2": _w((lambda *s: _rng.normal(s) * 0.05)(D) * 0.01),
    }

def reference(x, w1, b1, w2, b2):
    h = jnp.einsum("bsd,df->bsf", x, w1) + b1
    h = _gelu(h)
    return jnp.einsum("bsf,fd->bsd", h, w2) + b2
```

```python
import jax
import jax.numpy as jnp
from jax import lax
import jax.experimental.pallas as pl
import jax.experimental.pallas.tpu as pltpu

_NT = (((1,), (1,)), ((), ()))

_TM = 512
_W1_CHUNKS = (256, 512)
_OUT_SPLIT = 4


def _gelu(h):
    return jax.nn.gelu(h, approximate=True)


@jax.jit
def pallas_standalone__dense_activation_gelu__prompt_kernel(
    x: jax.Array,
    w1: jax.Array,
    b1: jax.Array,
    w2: jax.Array,
    b2: jax.Array,
):
    B, S, D = x.shape
    F = w1.shape[1]
    M = B * S
    tm = _TM
    assert M % tm == 0
    nt = M // tm
    osplit = _OUT_SPLIT
    om = tm // osplit
    bf16, f32 = jnp.bfloat16, jnp.float32

    chunks, start = [], 0
    for c in _W1_CHUNKS:
        chunks.append((start, c))
        start += c
    assert start < F
    chunks.append((start, F - start))
    nc = len(chunks)
    n_in = nt + nc + 3

    def kernel_function(x_hbm, w1t_hbm, b1_hbm, w2_hbm, b2_hbm, o_hbm,
                        x_v, w1_v, b1_v, w2_v, b2_v, o_v, h_v, in_sems, o_sems):
        def x_cp(i):
            return pltpu.make_async_copy(
                x_hbm.at[pl.ds(i * tm, tm)], x_v.at[pl.ds(i * tm, tm)], in_sems.at[i])

        def w1_cp(j):
            s, n = chunks[j]
            return pltpu.make_async_copy(
                w1t_hbm.at[pl.ds(s, n)], w1_v.at[pl.ds(s, n)], in_sems.at[nt + j])

        b1_cp = pltpu.make_async_copy(b1_hbm, b1_v, in_sems.at[nt + nc])
        b2_cp = pltpu.make_async_copy(b2_hbm, b2_v, in_sems.at[nt + nc + 1])
        w2_cp = pltpu.make_async_copy(w2_hbm, w2_v, in_sems.at[nt + nc + 2])

        def o_cp(i, k):
            r = i * tm + k * om
            return pltpu.make_async_copy(
                o_v.at[pl.ds(r, om)], o_hbm.at[pl.ds(r, om)], o_sems.at[i * osplit + k])

        x_cp(0).start()
        for j in range(nc):
            w1_cp(j).start()
            if j == 0:
                b1_cp.start()
        b2_cp.start()
        w2_cp.start()
        for i in range(1, nt):
            x_cp(i).start()

        def second_matmul(i, r, h_slab):
            b2_row = b2_v[...].astype(f32)[None, :]
            for k in range(osplit):
                o = jnp.dot(h_slab(k), w2_v[...], preferred_element_type=f32)
                o_v[pl.ds(r + k * om, om), :] = (o + b2_row).astype(bf16)
                o_cp(i, k).start()

        x_cp(0).wait()
        x0 = x_v[pl.ds(0, tm), :]
        for j, (s, n) in enumerate(chunks):
            w1_cp(j).wait()
            if j == 0:
                b1_cp.wait()
            hj = lax.dot_general(x0, w1_v[pl.ds(s, n), :], _NT, preferred_element_type=f32)
            hj = hj + b1_v[...].astype(f32)[None, s:s + n]
            h_v[:, s:s + n] = _gelu(hj).astype(bf16)
        b2_cp.wait()
        w2_cp.wait()
        second_matmul(0, 0, lambda k: h_v[pl.ds(k * om, om), :])

        def body(i, carry):
            x_cp(i).wait()
            r = pl.multiple_of(i * tm, tm)
            h = lax.dot_general(x_v[pl.ds(r, tm), :], w1_v[...], _NT, preferred_element_type=f32)
            h = _gelu(h + b1_v[...].astype(f32)[None, :]).astype(bf16)
            second_matmul(i, r, lambda k: h[k * om:(k + 1) * om, :])
            return carry

        lax.fori_loop(1, nt, body, 0)
        for i in range(nt):
            for k in range(osplit):
                o_cp(i, k).wait()

    hbm = pl.BlockSpec(memory_space=pl.ANY)
    out = pl.pallas_call(
        kernel_function,
        in_specs=[hbm] * 5,
        out_specs=hbm,
        out_shape=jax.ShapeDtypeStruct((M, D), x.dtype),
        scratch_shapes=[
            pltpu.VMEM((M, D), bf16),
            pltpu.VMEM((F, D), bf16),
            pltpu.VMEM((F,), bf16),
            pltpu.VMEM((F, D), bf16),
            pltpu.VMEM((D,), bf16),
            pltpu.VMEM((M, D), bf16),
            pltpu.VMEM((tm, F), bf16),
            pltpu.SemaphoreType.DMA((n_in,)),
            pltpu.SemaphoreType.DMA((nt * osplit,)),
        ],
        compiler_params=pltpu.CompilerParams(vmem_limit_bytes=64 * 1024 * 1024),
    )(x.reshape(M, D), w1.T, b1, w2, b2)
    return out.reshape(B, S, D)
```

```python
import jax
import jax.numpy as jnp
from jax import lax
import jax.experimental.pallas as pl
import jax.experimental.pallas.tpu as pltpu

_NT = (((1,), (1,)), ((), ()))

_HEAD = 512
_HEAD_CHUNKS = (128, 256, 512)
_HEAD_SLABS = (128, 256, 256, 256)
_TILES = ((256, 256), (512, 256, 256))
_COL_SPLIT = 512


def _gelu(h):
    return jax.nn.gelu(h, approximate=True)


@jax.jit
def pallas_standalone__dense_activation_gelu__prompt_kernel(
    x: jax.Array,
    w1: jax.Array,
    b1: jax.Array,
    w2: jax.Array,
    b2: jax.Array,
):
    B, S, D = x.shape
    F = w1.shape[1]
    M = B * S
    bf16, f32 = jnp.bfloat16, jnp.float32
    t0, csplit = _HEAD, _COL_SPLIT

    chunks, start = [], 0
    for c in _HEAD_CHUNKS:
        chunks.append((start, c))
        start += c
    assert start < F
    chunks.append((start, F - start))
    nc = len(chunks)

    tiles, start = [], t0
    for slabs in _TILES:
        tiles.append((start, sum(slabs), slabs))
        start += sum(slabs)
    assert start == M
    nl = len(tiles)
    nx = 1 + nl
    n_in = nx + 2 * nc + 2
    n_out = 2 + sum(len(t[2]) for t in tiles)

    def kernel_function(x_hbm, w1t_hbm, b1_hbm, w2_hbm, b2_hbm, o_hbm,
                        x_v, w1_v, b1_v, w2_v, b2_v, o_v, acc_v, b1c_v,
                        in_sems, out_sems):
        def x_cp(p):
            s, n = (0, t0) if p == 0 else tiles[p - 1][:2]
            return pltpu.make_async_copy(
                x_hbm.at[pl.ds(s, n)], x_v.at[pl.ds(s, n)], in_sems.at[p])

        def w1_cp(j):
            s, n = chunks[j]
            return pltpu.make_async_copy(
                w1t_hbm.at[pl.ds(s, n)], w1_v.at[pl.ds(s, n)], in_sems.at[nx + j])

        def w2_cp(j):
            s, n = chunks[j]
            return pltpu.make_async_copy(
                w2_hbm.at[pl.ds(s, n)], w2_v.at[pl.ds(s, n)], in_sems.at[nx + nc + j])

        b1_cp = pltpu.make_async_copy(b1_hbm, b1_v, in_sems.at[nx + 2 * nc])
        b2_cp = pltpu.make_async_copy(b2_hbm, b2_v, in_sems.at[nx + 2 * nc + 1])

        def out_rows(r, n, sem):
            return pltpu.make_async_copy(
                o_v.at[pl.ds(r, n)], o_hbm.at[pl.ds(r, n)], out_sems.at[sem])

        def out_cols(r, n, c, m, sem):
            return pltpu.make_async_copy(
                o_v.at[pl.ds(r, n), pl.ds(c, m)],
                o_hbm.at[pl.ds(r, n), pl.ds(c, m)], out_sems.at[sem])

        head_out = out_rows(0, t0, 0)
        tile_outs, sem = [], 1
        for i, (r, _, slabs) in enumerate(tiles):
            cps, off = [], 0
            for k, c in enumerate(slabs):
                if i == nl - 1 and k == len(slabs) - 1:
                    cps.append([out_cols(r + off, c, 0, csplit, sem),
                                out_cols(r + off, c, csplit, D - csplit, sem + 1)])
                    sem += 2
                else:
                    cps.append([out_rows(r + off, c, sem)])
                    sem += 1
                off += c
            tile_outs.append(cps)

        b1_cp.start()
        x_cp(0).start()
        for j in range(nc):
            w1_cp(j).start()
            w2_cp(j).start()
            if j == nc - 2:
                b2_cp.start()
        for p in range(1, nx):
            x_cp(p).start()

        def hidden_t(xt, s, n):
            ht = lax.dot_general(w1_v[pl.ds(s, n), :], xt, _NT, preferred_element_type=f32)
            bias = b1c_v[pl.ds(s, n), :]
            bias = jnp.concatenate([bias] * (xt.shape[0] // 128), axis=1)
            return _gelu(ht + bias).astype(bf16)

        def head_region(j):
            s, n = chunks[j]
            m = _HEAD_SLABS[j]
            ht = hidden_t(x_v[pl.ds(0, t0), :], s, n)
            for k in range(t0 // m):
                rows = pl.ds(k * m, m)
                p = jnp.dot(ht[:, k * m:(k + 1) * m].T, w2_v[pl.ds(s, n), :],
                            preferred_element_type=f32)
                if j > 0:
                    p = p + acc_v[rows, :]
                if j < nc - 1:
                    acc_v[rows, :] = p
                else:
                    o_v[rows, :] = (p + b2_v[...].astype(f32)[None, :]).astype(bf16)

        def head():
            b1_cp.wait()
            b1c_v[...] = jnp.broadcast_to(b1_v[...].astype(f32)[None, :], (128, F)).T
            x_cp(0).wait()
            for j in range(nc):
                w1_cp(j).wait()
                w2_cp(j).wait()
                if j == nc - 1:
                    b2_cp.wait()
                    x_cp(1).wait()
                head_region(j)
            head_out.start()

        def tile(i):
            r, n, slabs = tiles[i]
            b2_row = b2_v[...].astype(f32)[None, :]
            ht = hidden_t(x_v[pl.ds(r, n), :], 0, F)
            off = 0
            for k, c in enumerate(slabs):
                rows = pl.ds(r + off, c)
                o = jnp.dot(ht[:, off:off + c].T, w2_v[...], preferred_element_type=f32)
                o = (o + b2_row).astype(bf16)
                cps = tile_outs[i][k]
                if len(cps) == 1:
                    o_v[rows, :] = o
                    cps[0].start()
                else:
                    o_v[rows, 0:csplit] = o[:, :csplit]
                    cps[0].start()
                    o_v[rows, csplit:] = o[:, csplit:]
                    cps[1].start()
                off += c

        def part_a():
            head()
            tile(0)

        def part_b():
            for i in range(1, nl):
                x_cp(1 + i).wait()
            for i in range(1, nl):
                tile(i)

        def body(t, carry):
            pl.when(t == 0)(part_a)
            pl.when(t == 1)(part_b)
            return carry

        lax.fori_loop(0, 2, body, 0)

        head_out.wait()
        for cps in tile_outs:
            for slab_cps in cps:
                for cp in slab_cps:
                    cp.wait()

    hbm = pl.BlockSpec(memory_space=pl.ANY)
    out = pl.pallas_call(
        kernel_function,
        in_specs=[hbm] * 5,
        out_specs=hbm,
        out_shape=jax.ShapeDtypeStruct((M, D), x.dtype),
        scratch_shapes=[
            pltpu.VMEM((M, D), bf16),
            pltpu.VMEM((F, D), bf16),
            pltpu.VMEM((F,), bf16),
            pltpu.VMEM((F, D), bf16),
            pltpu.VMEM((D,), bf16),
            pltpu.VMEM((M, D), bf16),
            pltpu.VMEM((t0, D), f32),
            pltpu.VMEM((F, 128), f32),
            pltpu.SemaphoreType.DMA((n_in,)),
            pltpu.SemaphoreType.DMA((n_out,)),
        ],
        compiler_params=pltpu.CompilerParams(vmem_limit_bytes=64 * 1024 * 1024),
    )(x.reshape(M, D), w1.T, b1, w2, b2)
    return out.reshape(B, S, D)
```

```python
import jax
import jax.numpy as jnp
from jax import lax
import jax.experimental.pallas as pl
import jax.experimental.pallas.tpu as pltpu

_NT = (((1,), (1,)), ((), ()))

_HEAD = 512
_HEAD_CHUNKS = (128, 128, 128, 128, 256, 256, 256)
_HEAD_SLAB = 128
_TILES = ((256, 256), (256, 256), (256, 256))
_COL_SPLIT = 512


def _gelu(h):
    return jax.nn.gelu(h, approximate=True)


@jax.jit
def pallas_standalone__dense_activation_gelu__prompt_kernel(
    x: jax.Array,
    w1: jax.Array,
    b1: jax.Array,
    w2: jax.Array,
    b2: jax.Array,
):
    B, S, D = x.shape
    F = w1.shape[1]
    M = B * S
    bf16, f32 = jnp.bfloat16, jnp.float32
    t0, mh, csplit = _HEAD, _HEAD_SLAB, _COL_SPLIT

    chunks, start = [], 0
    for c in _HEAD_CHUNKS:
        chunks.append((start, c))
        start += c
    assert start < F
    chunks.append((start, F - start))
    nc = len(chunks)

    tiles, start = [], t0
    for slabs in _TILES:
        tiles.append((start, sum(slabs), slabs))
        start += sum(slabs)
    assert start == M
    nl = len(tiles)
    nx = 1 + nl
    n_in = nx + 2 * nc + 2

    def kernel_function(x_hbm, w1t_hbm, b1_hbm, w2_hbm, b2_hbm, o_hbm,
                        x_v, w1_v, b1_v, w2_v, b2_v, o_v, acc_v, b1c_v,
                        in_sems, out_sem):
        def x_cp(p):
            s, n = (0, t0) if p == 0 else tiles[p - 1][:2]
            return pltpu.make_async_copy(
                x_hbm.at[pl.ds(s, n)], x_v.at[pl.ds(s, n)], in_sems.at[p])

        def w1_cp(j):
            s, n = chunks[j]
            return pltpu.make_async_copy(
                w1t_hbm.at[pl.ds(s, n)], w1_v.at[pl.ds(s, n)], in_sems.at[nx + j])

        def w2_cp(j):
            s, n = chunks[j]
            return pltpu.make_async_copy(
                w2_hbm.at[pl.ds(s, n)], w2_v.at[pl.ds(s, n)], in_sems.at[nx + nc + j])

        b1_cp = pltpu.make_async_copy(b1_hbm, b1_v, in_sems.at[nx + 2 * nc])
        b2_cp = pltpu.make_async_copy(b2_hbm, b2_v, in_sems.at[nx + 2 * nc + 1])

        def out_rows(r, n):
            return pltpu.make_async_copy(
                o_v.at[pl.ds(r, n)], o_hbm.at[pl.ds(r, n)], out_sem)

        def out_cols(r, n, c, m):
            return pltpu.make_async_copy(
                o_v.at[pl.ds(r, n), pl.ds(c, m)],
                o_hbm.at[pl.ds(r, n), pl.ds(c, m)], out_sem)

        b1_cp.start()
        x_cp(0).start()
        for j in range(nc):
            w1_cp(j).start()
            if j == nc - 1:
                b2_cp.start()
            w2_cp(j).start()
        for p in range(1, nx):
            x_cp(p).start()

        def hidden_t(r, rows, s, n):
            ht = lax.dot_general(w1_v[pl.ds(s, n), :], x_v[pl.ds(r, rows), :], _NT,
                                 preferred_element_type=f32)
            bias = b1c_v[pl.ds(s, n), :]
            bias = jnp.concatenate([bias] * (rows // 128), axis=1)
            return _gelu(ht + bias).astype(bf16)

        def head_chunk(j):
            s, n = chunks[j]
            w1_cp(j).wait()
            ht = hidden_t(0, t0, s, n)
            w2_cp(j).wait()
            if j == nc - 1:
                b2_cp.wait()
            for k in range(t0 // mh):
                rows = pl.ds(k * mh, mh)
                p = jnp.dot(ht[:, k * mh:(k + 1) * mh].T, w2_v[pl.ds(s, n), :],
                            preferred_element_type=f32)
                if j > 0:
                    p = p + acc_v[rows, :]
                if j < nc - 1:
                    acc_v[rows, :] = p
                else:
                    o_v[rows, :] = (p + b2_v[...].astype(f32)[None, :]).astype(bf16)

        def tile(i):
            r, n, slabs = tiles[i]
            x_cp(1 + i).wait()
            b2_row = b2_v[...].astype(f32)[None, :]
            ht = hidden_t(r, n, 0, F)
            off = 0
            for k, c in enumerate(slabs):
                rows = pl.ds(r + off, c)
                o = jnp.dot(ht[:, off:off + c].T, w2_v[...], preferred_element_type=f32)
                o = (o + b2_row).astype(bf16)
                if i == nl - 1 and k == len(slabs) - 1:
                    o_v[rows, 0:csplit] = o[:, :csplit]
                    out_cols(r + off, c, 0, csplit).start()
                    o_v[rows, csplit:] = o[:, csplit:]
                    out_cols(r + off, c, csplit, D - csplit).start()
                else:
                    o_v[rows, :] = o
                    out_rows(r + off, c).start()
                off += c

        def setup():
            b1_cp.wait()
            b1c_v[...] = jnp.broadcast_to(b1_v[...].astype(f32)[None, :], (128, F)).T
            x_cp(0).wait()

        def main():
            for j in range(nc):
                head_chunk(j)
            out_rows(0, t0).start()
            for i in range(nl):
                tile(i)

        def body(t, carry):
            pl.when(t == 0)(setup)
            pl.when(t == 1)(main)
            return carry

        lax.fori_loop(0, 2, body, 0)

        pltpu.make_async_copy(o_v, o_v, out_sem).wait()

    hbm = pl.BlockSpec(memory_space=pl.ANY)
    out = pl.pallas_call(
        kernel_function,
        in_specs=[hbm] * 5,
        out_specs=hbm,
        out_shape=jax.ShapeDtypeStruct((M, D), x.dtype),
        scratch_shapes=[
            pltpu.VMEM((M, D), bf16),
            pltpu.VMEM((F, D), bf16),
            pltpu.VMEM((F,), bf16),
            pltpu.VMEM((F, D), bf16),
            pltpu.VMEM((D,), bf16),
            pltpu.VMEM((M, D), bf16),
            pltpu.VMEM((t0, D), f32),
            pltpu.VMEM((F, 128), f32),
            pltpu.SemaphoreType.DMA((n_in,)),
            pltpu.SemaphoreType.DMA,
        ],
        compiler_params=pltpu.CompilerParams(
            vmem_limit_bytes=64 * 1024 * 1024,
            disable_semaphore_checks=True,
            flags={"XLA_TPU_RESCHEDULE_DMA_DONES": True},
        ),
    )(x.reshape(M, D), w1.T, b1, w2, b2)
    return out.reshape(B, S, D)
```

```python
import jax
import jax.numpy as jnp
from jax import lax
import jax.experimental.pallas as pl
import jax.experimental.pallas.tpu as pltpu

_NT = (((1,), (1,)), ((), ()))

_HEAD = 512
_HEAD_CHUNKS = (64, 128, 256, 256, 512)
_HEAD_SLAB = 128
_TILES = ((1024, 256, 256),)
_COL_SPLIT = 512


def _gelu(h):
    return jax.nn.gelu(h, approximate=True)


@jax.jit
def pallas_standalone__dense_activation_gelu__prompt_kernel(
    x: jax.Array,
    w1: jax.Array,
    b1: jax.Array,
    w2: jax.Array,
    b2: jax.Array,
):
    B, S, D = x.shape
    F = w1.shape[1]
    M = B * S
    bf16, f32 = jnp.bfloat16, jnp.float32
    t0, mh, csplit = _HEAD, _HEAD_SLAB, _COL_SPLIT

    chunks, start = [], 0
    for c in _HEAD_CHUNKS:
        chunks.append((start, c))
        start += c
    assert start < F
    chunks.append((start, F - start))
    nc = len(chunks)

    tiles, start = [], t0
    for slabs in _TILES:
        tiles.append((start, sum(slabs), slabs))
        start += sum(slabs)
    assert start == M
    nl = len(tiles)
    nx = 1 + nl
    n_in = nx + 2 * nc + 2

    def kernel_function(x_hbm, w1t_hbm, b1_hbm, w2_hbm, b2_hbm, o_hbm,
                        x_v, w1_v, b1_v, w2_v, b2_v, o_v, acc_v, b1c_v,
                        in_sems, out_sem):
        def x_cp(p):
            s, n = (0, t0) if p == 0 else tiles[p - 1][:2]
            return pltpu.make_async_copy(
                x_hbm.at[pl.ds(s, n)], x_v.at[pl.ds(s, n)], in_sems.at[p])

        def w1_cp(j):
            s, n = chunks[j]
            return pltpu.make_async_copy(
                w1t_hbm.at[pl.ds(s, n)], w1_v.at[pl.ds(s, n)], in_sems.at[nx + j])

        def w2_cp(j):
            s, n = chunks[j]
            return pltpu.make_async_copy(
                w2_hbm.at[pl.ds(s, n)], w2_v.at[pl.ds(s, n)], in_sems.at[nx + nc + j])

        b1_cp = pltpu.make_async_copy(b1_hbm, b1_v, in_sems.at[nx + 2 * nc])
        b2_cp = pltpu.make_async_copy(b2_hbm, b2_v, in_sems.at[nx + 2 * nc + 1])

        def out_rows(r, n):
            return pltpu.make_async_copy(
                o_v.at[pl.ds(r, n)], o_hbm.at[pl.ds(r, n)], out_sem)

        def out_cols(r, n, c, m):
            return pltpu.make_async_copy(
                o_v.at[pl.ds(r, n), pl.ds(c, m)],
                o_hbm.at[pl.ds(r, n), pl.ds(c, m)], out_sem)

        b1_cp.start()
        for j in range(nc):
            w1_cp(j).start()
            if j == 0:
                x_cp(0).start()
            if j == nc - 1:
                b2_cp.start()
            w2_cp(j).start()
        for p in range(1, nx):
            x_cp(p).start()

        def hidden_t(r, rows, s, n):
            ht = lax.dot_general(w1_v[pl.ds(s, n), :], x_v[pl.ds(r, rows), :], _NT,
                                 preferred_element_type=f32)
            bias = b1c_v[pl.ds(s, n), :]
            bias = jnp.concatenate([bias] * (rows // 128), axis=1)
            return _gelu(ht + bias).astype(bf16)

        def head_chunk(j):
            s, n = chunks[j]
            w1_cp(j).wait()
            ht = hidden_t(0, t0, s, n)
            w2_cp(j).wait()
            if j == nc - 1:
                b2_cp.wait()
            for k in range(t0 // mh):
                rows = pl.ds(k * mh, mh)
                p = jnp.dot(ht[:, k * mh:(k + 1) * mh].T, w2_v[pl.ds(s, n), :],
                            preferred_element_type=f32)
                if j > 0:
                    p = p + acc_v[rows, :]
                if j < nc - 1:
                    acc_v[rows, :] = p
                else:
                    o_v[rows, :] = (p + b2_v[...].astype(f32)[None, :]).astype(bf16)

        def tile(i):
            r, n, slabs = tiles[i]
            x_cp(1 + i).wait()
            b2_row = b2_v[...].astype(f32)[None, :]
            ht = hidden_t(r, n, 0, F)
            off = 0
            for k, c in enumerate(slabs):
                rows = pl.ds(r + off, c)
                o = jnp.dot(ht[:, off:off + c].T, w2_v[...], preferred_element_type=f32)
                o = (o + b2_row).astype(bf16)
                if i == nl - 1 and k == len(slabs) - 1:
                    o_v[rows, 0:csplit] = o[:, :csplit]
                    out_cols(r + off, c, 0, csplit).start()
                    o_v[rows, csplit:] = o[:, csplit:]
                    out_cols(r + off, c, csplit, D - csplit).start()
                else:
                    o_v[rows, :] = o
                    out_rows(r + off, c).start()
                off += c

        def setup():
            b1_cp.wait()
            b1c_v[...] = jnp.broadcast_to(b1_v[...].astype(f32)[None, :], (128, F)).T

        def main():
            x_cp(0).wait()
            for j in range(nc):
                head_chunk(j)
            out_rows(0, t0).start()
            for i in range(nl):
                tile(i)

        def body(t, carry):
            pl.when(t == 0)(setup)
            pl.when(t == 1)(main)
            return carry

        lax.fori_loop(0, 2, body, 0)

        pltpu.make_async_copy(o_v, o_v, out_sem).wait()

    hbm = pl.BlockSpec(memory_space=pl.ANY)
    out = pl.pallas_call(
        kernel_function,
        in_specs=[hbm] * 5,
        out_specs=hbm,
        out_shape=jax.ShapeDtypeStruct((M, D), x.dtype),
        scratch_shapes=[
            pltpu.VMEM((M, D), bf16),
            pltpu.VMEM((F, D), bf16),
            pltpu.VMEM((F,), bf16),
            pltpu.VMEM((F, D), bf16),
            pltpu.VMEM((D,), bf16),
            pltpu.VMEM((M, D), bf16),
            pltpu.VMEM((t0, D), f32),
            pltpu.VMEM((F, 128), f32),
            pltpu.SemaphoreType.DMA((n_in,)),
            pltpu.SemaphoreType.DMA,
        ],
        compiler_params=pltpu.CompilerParams(
            vmem_limit_bytes=64 * 1024 * 1024,
            disable_semaphore_checks=True,
            flags={"XLA_TPU_RESCHEDULE_DMA_DONES": True},
        ),
    )(x.reshape(M, D), w1.T, b1, w2, b2)
    return out.reshape(B, S, D)
```

```python
import jax
import jax.numpy as jnp
from jax import lax
import jax.experimental.pallas as pl
import jax.experimental.pallas.tpu as pltpu

_NT = (((1,), (1,)), ((), ()))

_HEAD = 512
_K_STEPS = (128, 128, 128, 256)
_ROW_CHUNKS = (
    (128, 128, 256, 256, 384, 576),
    (512, 1216),
    (864, 864),
    (448, 256, 512, 512),
)
_HEAD_SLAB = 128
_TAIL_SLABS = (1024, 256, 256)
_COL_SPLIT = 512


def _gelu(h):
    return jax.nn.gelu(h, approximate=True)


def _spans(sizes):
    out, start = [], 0
    for n in sizes:
        out.append((start, n))
        start += n
    return out, start


@jax.jit
def pallas_standalone__dense_activation_gelu__prompt_kernel(
    x: jax.Array,
    w1: jax.Array,
    b1: jax.Array,
    w2: jax.Array,
    b2: jax.Array,
):
    B, S, D = x.shape
    F = w1.shape[1]
    M = B * S
    bf16, f32 = jnp.bfloat16, jnp.float32
    t0, mh, csplit = _HEAD, _HEAD_SLAB, _COL_SPLIT
    t1 = M - t0

    k_steps, total = _spans(_K_STEPS)
    assert total == D
    nk = len(k_steps)
    row_chunks = []
    for sizes in _ROW_CHUNKS:
        spans, total = _spans(sizes)
        assert total == F
        row_chunks.append(spans)
    assert len(row_chunks) == nk
    last_chunks = row_chunks[-1]
    nd = len(last_chunks)
    tail_slabs, total = _spans(_TAIL_SLABS)
    assert total == t1

    order = [("b1",)]
    for k in range(nk):
        ws = [("w", k, j) for j in range(len(row_chunks[k]))]
        if k == 0:
            order += [("x", 0)] + ws[:4] + [("x", 1)] + ws[4:]
        elif k < nk - 1:
            order += ws + [("x", k + 1)]
        else:
            for j, w in enumerate(ws):
                order.append(w)
                if j == nd - 1:
                    order.append(("b2",))
                order.append(("d", j))
    order.append(("t",))
    sem_of = {name: i for i, name in enumerate(order)}

    def kernel_function(x_hbm, w1t_hbm, b1_hbm, w2_hbm, b2_hbm, o_hbm,
                        x_v, w1_v, b1_v, w2_v, b2_v, o_v, acc_v, pre_v, b1c_v,
                        in_sems, out_sem):
        def in_copy(name):
            sem = in_sems.at[sem_of[name]]
            kind = name[0]
            if kind == "b1":
                return pltpu.make_async_copy(b1_hbm, b1_v, sem)
            if kind == "b2":
                return pltpu.make_async_copy(b2_hbm, b2_v, sem)
            if kind == "t":
                idx = pl.ds(t0, t1)
                return pltpu.make_async_copy(x_hbm.at[idx], x_v.at[idx], sem)
            if kind == "d":
                idx = pl.ds(*last_chunks[name[1]])
                return pltpu.make_async_copy(w2_hbm.at[idx], w2_v.at[idx], sem)
            cols = pl.ds(*k_steps[name[1]])
            if kind == "x":
                idx = (pl.ds(0, t0), cols)
                return pltpu.make_async_copy(x_hbm.at[idx], x_v.at[idx], sem)
            idx = (pl.ds(*row_chunks[name[1]][name[2]]), cols)
            return pltpu.make_async_copy(w1t_hbm.at[idx], w1_v.at[idx], sem)

        def out_copy(r, n, c=0, m=D):
            idx = (pl.ds(r, n), pl.ds(c, m))
            return pltpu.make_async_copy(o_v.at[idx], o_hbm.at[idx], out_sem)

        for name in order:
            in_copy(name).start()

        def bias_t(s, n, rows):
            return jnp.concatenate([b1c_v[pl.ds(s, n), :]] * (rows // 128), axis=1)

        def head_second_matmul(j, ht):
            s, n = last_chunks[j]
            in_copy(("d", j)).wait()
            if j == nd - 1:
                in_copy(("b2",)).wait()
            for i in range(t0 // mh):
                rows = pl.ds(i * mh, mh)
                p = jnp.dot(ht[:, i * mh:(i + 1) * mh].T, w2_v[pl.ds(s, n), :],
                            preferred_element_type=f32)
                if j > 0:
                    p = p + acc_v[rows, :]
                if j < nd - 1:
                    acc_v[rows, :] = p
                else:
                    o_v[rows, :] = (p + b2_v[...].astype(f32)[None, :]).astype(bf16)

        def head():
            for k, (c, kn) in enumerate(k_steps):
                in_copy(("x", k)).wait()
                xk = x_v[pl.ds(0, t0), pl.ds(c, kn)]
                for j, (s, n) in enumerate(row_chunks[k]):
                    in_copy(("w", k, j)).wait()
                    part = lax.dot_general(w1_v[pl.ds(s, n), pl.ds(c, kn)], xk, _NT,
                                           preferred_element_type=f32)
                    rows = pl.ds(s, n)
                    if k == 0:
                        pre_v[rows, :] = part + bias_t(s, n, t0)
                    elif k < nk - 1:
                        pre_v[rows, :] += part
                    else:
                        ht = _gelu(pre_v[rows, :] + part).astype(bf16)
                        head_second_matmul(j, ht)
            out_copy(0, t0).start()

        def tail():
            in_copy(("t",)).wait()
            ht = lax.dot_general(w1_v[...], x_v[pl.ds(t0, t1), :], _NT,
                                 preferred_element_type=f32)
            ht = _gelu(ht + bias_t(0, F, t1)).astype(bf16)
            b2_row = b2_v[...].astype(f32)[None, :]
            for i, (off, n) in enumerate(tail_slabs):
                r = t0 + off
                o = jnp.dot(ht[:, off:off + n].T, w2_v[...], preferred_element_type=f32)
                o = (o + b2_row).astype(bf16)
                if i < len(tail_slabs) - 1:
                    o_v[pl.ds(r, n), :] = o
                    out_copy(r, n).start()
                else:
                    o_v[pl.ds(r, n), 0:csplit] = o[:, :csplit]
                    out_copy(r, n, 0, csplit).start()
                    o_v[pl.ds(r, n), csplit:] = o[:, csplit:]
                    out_copy(r, n, csplit, D - csplit).start()

        def setup():
            in_copy(("b1",)).wait()
            b1c_v[...] = jnp.broadcast_to(b1_v[...].astype(f32)[None, :], (128, F)).T

        def main():
            head()
            tail()

        def body(t, carry):
            pl.when(t == 0)(setup)
            pl.when(t == 1)(main)
            return carry

        lax.fori_loop(0, 2, body, 0)

        pltpu.make_async_copy(o_v, o_v, out_sem).wait()

    hbm = pl.BlockSpec(memory_space=pl.ANY)
    out = pl.pallas_call(
        kernel_function,
        in_specs=[hbm] * 5,
        out_specs=hbm,
        out_shape=jax.ShapeDtypeStruct((M, D), x.dtype),
        scratch_shapes=[
            pltpu.VMEM((M, D), bf16),
            pltpu.VMEM((F, D), bf16),
            pltpu.VMEM((F,), bf16),
            pltpu.VMEM((F, D), bf16),
            pltpu.VMEM((D,), bf16),
            pltpu.VMEM((M, D), bf16),
            pltpu.VMEM((t0, D), f32),
            pltpu.VMEM((F, t0), f32),
            pltpu.VMEM((F, 128), f32),
            pltpu.SemaphoreType.DMA((len(order),)),
            pltpu.SemaphoreType.DMA(()),
        ],
        compiler_params=pltpu.CompilerParams(
            vmem_limit_bytes=64 * 1024 * 1024,
            disable_semaphore_checks=True,
            flags={"XLA_TPU_RESCHEDULE_DMA_DONES": True},
        ),
    )(x.reshape(M, D), w1.T, b1, w2, b2)
    return out.reshape(B, S, D)
```

```python
import jax
import jax.numpy as jnp
from jax import lax
import jax.experimental.pallas as pl
import jax.experimental.pallas.tpu as pltpu

_NT = (((1,), (1,)), ((), ()))

_HEAD = 512
_K_STEPS = (128, 128, 128, 256)
_ROW_CHUNKS = (
    (128, 128, 256, 256, 384, 576),
    (512, 1216),
    (864, 864),
    (448, 256, 512, 512),
)
_HEAD_SLAB = 128
_TAIL_SLABS = (1024, 256, 256)
_COL_SPLIT = 512
_LAST_ROWS = (96, 64, 48, 32, 16)


def _gelu(h):
    return jax.nn.gelu(h, approximate=True)


def _spans(sizes):
    out, start = [], 0
    for n in sizes:
        out.append((start, n))
        start += n
    return out, start


@jax.jit
def pallas_standalone__dense_activation_gelu__prompt_kernel(
    x: jax.Array,
    w1: jax.Array,
    b1: jax.Array,
    w2: jax.Array,
    b2: jax.Array,
):
    B, S, D = x.shape
    F = w1.shape[1]
    M = B * S
    bf16, f32 = jnp.bfloat16, jnp.float32
    t0, mh, csplit = _HEAD, _HEAD_SLAB, _COL_SPLIT
    t1 = M - t0

    k_steps, total = _spans(_K_STEPS)
    assert total == D
    nk = len(k_steps)
    row_chunks = []
    for sizes in _ROW_CHUNKS:
        spans, total = _spans(sizes)
        assert total == F
        row_chunks.append(spans)
    assert len(row_chunks) == nk
    last_chunks = row_chunks[-1]
    nd = len(last_chunks)
    tail_slabs, total = _spans(_TAIL_SLABS)
    assert total == t1
    last_rows, total = _spans(_LAST_ROWS)
    assert total == _TAIL_SLABS[-1]

    order = [("b1",)]
    for k in range(nk):
        ws = [("w", k, j) for j in range(len(row_chunks[k]))]
        if k == 0:
            order += [("x", 0)] + ws[:4] + [("x", 1)] + ws[4:]
        elif k < nk - 1:
            order += ws + [("x", k + 1)]
        else:
            for j, w in enumerate(ws):
                order.append(w)
                if j == nd - 1:
                    order.append(("b2",))
                order.append(("d", j))
    order.append(("t",))
    sem_of = {name: i for i, name in enumerate(order)}

    def kernel_function(x_hbm, w1t_hbm, b1_hbm, w2_hbm, b2_hbm, o_hbm,
                        x_v, w1_v, b1_v, w2_v, b2_v, o_v, acc_v, pre_v, b1c_v,
                        in_sems, out_sem):
        def in_copy(name):
            sem = in_sems.at[sem_of[name]]
            kind = name[0]
            if kind == "b1":
                return pltpu.make_async_copy(b1_hbm, b1_v, sem)
            if kind == "b2":
                return pltpu.make_async_copy(b2_hbm, b2_v, sem)
            if kind == "t":
                idx = pl.ds(t0, t1)
                return pltpu.make_async_copy(x_hbm.at[idx], x_v.at[idx], sem)
            if kind == "d":
                idx = pl.ds(*last_chunks[name[1]])
                return pltpu.make_async_copy(w2_hbm.at[idx], w2_v.at[idx], sem)
            cols = pl.ds(*k_steps[name[1]])
            if kind == "x":
                idx = (pl.ds(0, t0), cols)
                return pltpu.make_async_copy(x_hbm.at[idx], x_v.at[idx], sem)
            idx = (pl.ds(*row_chunks[name[1]][name[2]]), cols)
            return pltpu.make_async_copy(w1t_hbm.at[idx], w1_v.at[idx], sem)

        def out_copy(r, n, c=0, m=D):
            idx = (pl.ds(r, n), pl.ds(c, m))
            return pltpu.make_async_copy(o_v.at[idx], o_hbm.at[idx], out_sem)

        for name in order:
            in_copy(name).start()

        def bias_t(s, n, rows):
            return jnp.concatenate([b1c_v[pl.ds(s, n), :]] * (rows // 128), axis=1)

        def head_second_matmul(j, ht):
            s, n = last_chunks[j]
            in_copy(("d", j)).wait()
            if j == nd - 1:
                in_copy(("b2",)).wait()
            for i in range(t0 // mh):
                rows = pl.ds(i * mh, mh)
                p = jnp.dot(ht[:, i * mh:(i + 1) * mh].T, w2_v[pl.ds(s, n), :],
                            preferred_element_type=f32)
                if j > 0:
                    p = p + acc_v[rows, :]
                if j < nd - 1:
                    acc_v[rows, :] = p
                else:
                    o_v[rows, :] = (p + b2_v[...].astype(f32)[None, :]).astype(bf16)

        def head():
            for k, (c, kn) in enumerate(k_steps):
                in_copy(("x", k)).wait()
                xk = x_v[pl.ds(0, t0), pl.ds(c, kn)]
                for j, (s, n) in enumerate(row_chunks[k]):
                    in_copy(("w", k, j)).wait()
                    part = lax.dot_general(w1_v[pl.ds(s, n), pl.ds(c, kn)], xk, _NT,
                                           preferred_element_type=f32)
                    rows = pl.ds(s, n)
                    if k == 0:
                        pre_v[rows, :] = part + bias_t(s, n, t0)
                    elif k < nk - 1:
                        pre_v[rows, :] += part
                    else:
                        ht = _gelu(pre_v[rows, :] + part).astype(bf16)
                        head_second_matmul(j, ht)
            out_copy(0, t0).start()

        def tail():
            in_copy(("t",)).wait()
            ht = lax.dot_general(w1_v[...], x_v[pl.ds(t0, t1), :], _NT,
                                 preferred_element_type=f32)
            ht = _gelu(ht + bias_t(0, F, t1)).astype(bf16)
            b2_row = b2_v[...].astype(f32)[None, :]
            for i, (off, n) in enumerate(tail_slabs):
                r = t0 + off
                o = jnp.dot(ht[:, off:off + n].T, w2_v[...], preferred_element_type=f32)
                o = (o + b2_row).astype(bf16)
                if i < len(tail_slabs) - 1:
                    o_v[pl.ds(r, n), :] = o
                    out_copy(r, n).start()
                else:
                    o_v[pl.ds(r, n), 0:csplit] = o[:, :csplit]
                    out_copy(r, n, 0, csplit).start()
                    for a, q in last_rows:
                        o_v[pl.ds(r + a, q), csplit:] = o[a:a + q, csplit:]
                        out_copy(r + a, q, csplit, D - csplit).start()

        def setup():
            in_copy(("b1",)).wait()
            b1c_v[...] = jnp.broadcast_to(b1_v[...].astype(f32)[None, :], (128, F)).T

        def main():
            head()
            tail()

        def body(t, carry):
            pl.when(t == 0)(setup)
            pl.when(t == 1)(main)
            return carry

        lax.fori_loop(0, 2, body, 0)

        pltpu.make_async_copy(o_v, o_v, out_sem).wait()

    hbm = pl.BlockSpec(memory_space=pl.ANY)
    out = pl.pallas_call(
        kernel_function,
        in_specs=[hbm] * 5,
        out_specs=hbm,
        out_shape=jax.ShapeDtypeStruct((M, D), x.dtype),
        scratch_shapes=[
            pltpu.VMEM((M, D), bf16),
            pltpu.VMEM((F, D), bf16),
            pltpu.VMEM((F,), bf16),
            pltpu.VMEM((F, D), bf16),
            pltpu.VMEM((D,), bf16),
            pltpu.VMEM((M, D), bf16),
            pltpu.VMEM((t0, D), f32),
            pltpu.VMEM((F, t0), f32),
            pltpu.VMEM((F, 128), f32),
            pltpu.SemaphoreType.DMA((len(order),)),
            pltpu.SemaphoreType.DMA(()),
        ],
        compiler_params=pltpu.CompilerParams(
            vmem_limit_bytes=64 * 1024 * 1024,
            disable_semaphore_checks=True,
            flags={"XLA_TPU_RESCHEDULE_DMA_DONES": True},
        ),
    )(x.reshape(M, D), w1.T, b1, w2, b2)
    return out.reshape(B, S, D)
```

```python
import jax
import jax.numpy as jnp
from jax import lax
import jax.experimental.pallas as pl
import jax.experimental.pallas.tpu as pltpu

_NT = (((1,), (1,)), ((), ()))

_HEAD = 512
_K_STEPS = (128, 128, 128, 256)
_ROW_CHUNKS = (
    (128, 128, 256, 256, 384, 256, 320),
    (384, 576, 768),
    (864, 864),
    (320, 384, 512, 512),
)
_HEAD_SLAB = 256
_TAIL_SLABS = (1024, 256, 256)
_COL_SPLIT = 512
_LAST_ROWS = (96, 64, 48, 32, 16)


def _gelu(h):
    return jax.nn.gelu(h, approximate=True)


def _spans(sizes):
    out, start = [], 0
    for n in sizes:
        out.append((start, n))
        start += n
    return out, start


@jax.jit
def pallas_standalone__dense_activation_gelu__prompt_kernel(
    x: jax.Array,
    w1: jax.Array,
    b1: jax.Array,
    w2: jax.Array,
    b2: jax.Array,
):
    B, S, D = x.shape
    F = w1.shape[1]
    M = B * S
    bf16, f32 = jnp.bfloat16, jnp.float32
    t0, mh, csplit = _HEAD, _HEAD_SLAB, _COL_SPLIT
    t1 = M - t0

    k_steps, total = _spans(_K_STEPS)
    assert total == D
    nk = len(k_steps)
    row_chunks = []
    for sizes in _ROW_CHUNKS:
        spans, total = _spans(sizes)
        assert total == F
        row_chunks.append(spans)
    assert len(row_chunks) == nk
    last_chunks = row_chunks[-1]
    nd = len(last_chunks)
    tail_slabs, total = _spans(_TAIL_SLABS)
    assert total == t1
    last_rows, total = _spans(_LAST_ROWS)
    assert total == _TAIL_SLABS[-1]

    order = [("b1",)]
    for k in range(nk):
        ws = [("w", k, j) for j in range(len(row_chunks[k]))]
        if k == 0:
            order.append(("x", 0))
        if k < nk - 1:
            order += ws + [("x", k + 1)]
        else:
            for j, w in enumerate(ws):
                order.append(w)
                if j == nd - 1:
                    order.append(("b2",))
                order.append(("d", j))
    order.append(("t",))
    sem_of = {name: i for i, name in enumerate(order)}

    def kernel_function(x_hbm, w1t_hbm, b1_hbm, w2_hbm, b2_hbm, o_hbm,
                        x_v, w1_v, b1_v, w2_v, b2_v, o_v, acc_v, pre_v, b1c_v,
                        in_sems, out_sem):
        def in_copy(name):
            sem = in_sems.at[sem_of[name]]
            kind = name[0]
            if kind == "b1":
                return pltpu.make_async_copy(b1_hbm, b1_v, sem)
            if kind == "b2":
                return pltpu.make_async_copy(b2_hbm, b2_v, sem)
            if kind == "t":
                idx = pl.ds(t0, t1)
                return pltpu.make_async_copy(x_hbm.at[idx], x_v.at[idx], sem)
            if kind == "d":
                idx = pl.ds(*last_chunks[name[1]])
                return pltpu.make_async_copy(w2_hbm.at[idx], w2_v.at[idx], sem)
            cols = pl.ds(*k_steps[name[1]])
            if kind == "x":
                idx = (pl.ds(0, t0), cols)
                return pltpu.make_async_copy(x_hbm.at[idx], x_v.at[idx], sem)
            idx = (pl.ds(*row_chunks[name[1]][name[2]]), cols)
            return pltpu.make_async_copy(w1t_hbm.at[idx], w1_v.at[idx], sem)

        def out_copy(r, n, c=0, m=D):
            idx = (pl.ds(r, n), pl.ds(c, m))
            return pltpu.make_async_copy(o_v.at[idx], o_hbm.at[idx], out_sem)

        for name in order:
            in_copy(name).start()

        def bias_t(s, n, rows):
            return jnp.concatenate([b1c_v[pl.ds(s, n), :]] * (rows // 128), axis=1)

        def head_second_matmul(j, ht):
            s, n = last_chunks[j]
            in_copy(("d", j)).wait()
            if j == nd - 1:
                in_copy(("b2",)).wait()
            for i in range(t0 // mh):
                rows = pl.ds(i * mh, mh)
                p = jnp.dot(ht[:, i * mh:(i + 1) * mh].T, w2_v[pl.ds(s, n), :],
                            preferred_element_type=f32)
                if j > 0:
                    p = p + acc_v[rows, :]
                if j < nd - 1:
                    acc_v[rows, :] = p
                else:
                    o_v[rows, :] = (p + b2_v[...].astype(f32)[None, :]).astype(bf16)

        def head():
            for k, (c, kn) in enumerate(k_steps):
                in_copy(("x", k)).wait()
                xk = x_v[pl.ds(0, t0), pl.ds(c, kn)]
                for j, (s, n) in enumerate(row_chunks[k]):
                    in_copy(("w", k, j)).wait()
                    part = lax.dot_general(w1_v[pl.ds(s, n), pl.ds(c, kn)], xk, _NT,
                                           preferred_element_type=f32)
                    rows = pl.ds(s, n)
                    if k == 0:
                        pre_v[rows, :] = part + bias_t(s, n, t0)
                    elif k < nk - 1:
                        pre_v[rows, :] += part
                    else:
                        ht = _gelu(pre_v[rows, :] + part).astype(bf16)
                        head_second_matmul(j, ht)
            out_copy(0, t0).start()

        def tail():
            in_copy(("t",)).wait()
            ht = lax.dot_general(w1_v[...], x_v[pl.ds(t0, t1), :], _NT,
                                 preferred_element_type=f32)
            ht = _gelu(ht + bias_t(0, F, t1)).astype(bf16)
            b2_row = b2_v[...].astype(f32)[None, :]
            for i, (off, n) in enumerate(tail_slabs):
                r = t0 + off
                o = jnp.dot(ht[:, off:off + n].T, w2_v[...], preferred_element_type=f32)
                o = (o + b2_row).astype(bf16)
                if i < len(tail_slabs) - 1:
                    o_v[pl.ds(r, n), :] = o
                    out_copy(r, n).start()
                else:
                    o_v[pl.ds(r, n), 0:csplit] = o[:, :csplit]
                    out_copy(r, n, 0, csplit).start()
                    for a, q in last_rows:
                        o_v[pl.ds(r + a, q), csplit:] = o[a:a + q, csplit:]
                        out_copy(r + a, q, csplit, D - csplit).start()

        def setup():
            in_copy(("b1",)).wait()
            b1c_v[...] = jnp.broadcast_to(b1_v[...].astype(f32)[None, :], (128, F)).T

        def main():
            head()
            tail()

        def body(t, carry):
            pl.when(t == 0)(setup)
            pl.when(t == 1)(main)
            return carry

        lax.fori_loop(0, 2, body, 0)

        pltpu.make_async_copy(o_v, o_v, out_sem).wait()

    hbm = pl.BlockSpec(memory_space=pl.ANY)
    out = pl.pallas_call(
        kernel_function,
        in_specs=[hbm] * 5,
        out_specs=hbm,
        out_shape=jax.ShapeDtypeStruct((M, D), x.dtype),
        scratch_shapes=[
            pltpu.VMEM((M, D), bf16),
            pltpu.VMEM((F, D), bf16),
            pltpu.VMEM((F,), bf16),
            pltpu.VMEM((F, D), bf16),
            pltpu.VMEM((D,), bf16),
            pltpu.VMEM((M, D), bf16),
            pltpu.VMEM((t0, D), f32),
            pltpu.VMEM((F, t0), f32),
            pltpu.VMEM((F, 128), f32),
            pltpu.SemaphoreType.DMA((len(order),)),
            pltpu.SemaphoreType.DMA(()),
        ],
        compiler_params=pltpu.CompilerParams(
            vmem_limit_bytes=64 * 1024 * 1024,
            disable_semaphore_checks=True,
            flags={"XLA_TPU_RESCHEDULE_DMA_DONES": True},
        ),
    )(x.reshape(M, D), w1.T, b1, w2, b2)
    return out.reshape(B, S, D)
```
